```python
import os as _os
_os.environ.setdefault("JAX_PLATFORMS", "cpu")
import jax
import jax.numpy as jnp

def _softmax(x, axis=-1):
    return jax.nn.softmax(x, axis=axis)
def _gelu(x):
    return jax.nn.gelu(x, approximate=True)
def _silu(x):
    return jax.nn.silu(x)
def _sigmoid(x):
    return jax.nn.sigmoid(x)
def _layernorm(x, axis=-1, eps=1e-5):
    m = jnp.mean(x, axis=axis, keepdims=True)
    v = jnp.var(x, axis=axis, keepdims=True)
    return (x - m) / jnp.sqrt(v + eps)
def _scatter_add(tgt, idx, src, axis=0):
    return tgt.at[idx].add(src)
def _segment_sum(src, seg, n):
    return jax.ops.segment_sum(src, seg, n)
class _Rng:
    def __init__(self, key):
        self._k = key
    def _next(self):
        self._k, sub = jax.random.split(self._k)
        return sub
    def normal(self, shape):
        return jax.random.normal(self._next(), shape, dtype=jnp.bfloat16)
    def randint(self, lo, hi, shape):
        return jax.random.randint(self._next(), shape, lo, hi, dtype=jnp.int32)
    def uniform(self, shape, lo=0.0, hi=1.0):
        return jax.random.uniform(self._next(), shape, jnp.bfloat16, lo, hi)
    def permutation(self, n):
        return jax.random.permutation(self._next(), n)


kernel_name = 'concat_heads__sliding_block_cached__compressed_kv_cla__decode'

def setup_inputs():
    _rng = _Rng(jax.random.key(int.from_bytes(__import__("os").urandom(4), "little")))
    _w = (lambda a: (lambda t: t.astype(jnp.bfloat16) if jnp.issubdtype(t.dtype, jnp.floating) else t)(jnp.asarray(a)))
    def _A_setup():
        B, Sq, D = 1, 1, 512
        Hq, Hkv, Sk, Dh = 32, 32, 4096, 128
        assert Hq % Hkv == 0, (Hq, Hkv)
        return {
            "x": _w((lambda *s: _rng.normal(s) * 0.8)(B, Sq, D)),
            "k_cache": _w((lambda *s: _rng.normal(s) * 0.8)(B, Hkv, Sk, Dh)),
            "v_cache": _w((lambda *s: _rng.normal(s) * 0.05)(B, Hkv, Sk, Dh)),
            "wq": _w((lambda *s: _rng.normal(s) * 0.8)(D, Hq * Dh) * (D ** -0.5)),
            "wo": _w((lambda *s: _rng.normal(s) * 0.05)(Hq * Dh, D) * ((Hq * Dh) ** -0.5)),
        }
    _A_in = _A_setup()

    def _B_setup():
        B, H, Sq, Sk, D, M = 1, 32, 1, 4096, 128, 512
        Dc = 4 * D
        return {
            "x": _w((lambda *s: _rng.normal(s) * 1.6)(B, Sq, M)),
            "c_kv": _w((lambda *s: _rng.normal(s) * 0.1)(B, Sk, Dc)),
            "w_q": _w((lambda *s: _rng.normal(s) * 1.6)(M, H, D) * (M ** -0.5)),
            "w_uk": _w((lambda *s: _rng.normal(s) * 1.6)(Dc, H, D) * (Dc ** -0.5)),
            "w_uv": _w((lambda *s: _rng.normal(s) * 0.1)(Dc, H, D) * (Dc ** -0.5)),
            "w_o": _w((lambda *s: _rng.normal(s) * 0.1)(H, D, M) * ((H * D) ** -0.5)),
        }
    _B_in = _B_setup()

    return {
        "A_x": _A_in["x"],
        "A_k_cache": _A_in["k_cache"],
        "A_v_cache": _A_in["v_cache"],
        "A_wq": _A_in["wq"],
        "A_wo": _A_in["wo"],
        "B_x": _B_in["x"],
        "B_c_kv": _B_in["c_kv"],
        "B_w_q": _B_in["w_q"],
        "B_w_uk": _B_in["w_uk"],
        "B_w_uv": _B_in["w_uv"],
        "B_w_o": _B_in["w_o"],
    }

def reference(A_x, A_k_cache, A_v_cache, A_wq, A_wo, B_x, B_c_kv, B_w_q, B_w_uk, B_w_uv, B_w_o):
    def _A_ref(x, k_cache, v_cache, wq, wo):
        B, Sq, D = x.shape
        Hq, Dh = 32, 128
        Hkv, Sk = k_cache.shape[1], k_cache.shape[2]
        W = min(4096, max(256, Sk // 4))
        rep = Hq // Hkv
        q = (lambda x, *d: x.transpose(*d))((x @ wq).reshape(B, Sq, Hq, Dh), 0, 2, 1, 3)
        k = jnp.repeat(k_cache[:, :, Sk - W:, :], rep, axis=1)
        v = jnp.repeat(v_cache[:, :, Sk - W:, :], rep, axis=1)
        scores = jnp.einsum("bhqd,bhkd->bhqk", q, k) * (Dh ** -0.5)
        p = _softmax(scores, axis=-1)
        o = jnp.einsum("bhqk,bhkd->bhqd", p, v)
        return (lambda x, *d: x.transpose(*d))(o, 0, 2, 1, 3).reshape(B, Sq, Hq * Dh) @ wo

    def _B_ref(x, c_kv, w_q, w_uk, w_uv, w_o):
        B, Sq, M = x.shape[0], x.shape[1], x.shape[2]
        Sk = c_kv.shape[1]
        H, D = w_q.shape[1], w_q.shape[2]
        q = jnp.einsum("bqm,mhd->bhqd", x, w_q)
        k = jnp.einsum("bkc,chd->bhkd", c_kv, w_uk)
        v = jnp.einsum("bkc,chd->bhkd", c_kv, w_uv)
        scores = jnp.einsum("bhqd,bhkd->bhqk", q, k) * (D ** -0.5)
        off = Sk - Sq
        qi = jnp.arange(Sq)[:, None]
        kj = jnp.arange(Sk)[None, :]
        cmask = kj <= (qi + off)
        scores = jnp.where(cmask[None, None], scores, -1e9)
        p = _softmax(scores, axis=-1)
        ctx = jnp.einsum("bhqk,bhkd->bhqd", p, v)
        return jnp.einsum("bhqd,hdm->bqm", ctx, w_o)

    a = _A_ref(A_x, A_k_cache, A_v_cache, A_wq, A_wo)
    b = _B_ref(B_x, B_c_kv, B_w_q, B_w_uk, B_w_uv, B_w_o)
    return jnp.concatenate([a, b], axis=-1)
```

```python
import jax
import jax.numpy as jnp
from jax import lax
import jax.experimental.pallas as pl
import jax.experimental.pallas.tpu as pltpu

BF = jnp.bfloat16
F32 = jnp.float32
LANES = 128
CW = 1024
KB = 512
WO_SPLIT = (20, 8, 3, 1)


def _dot(a, b):
    return jnp.dot(a, b, preferred_element_type=F32)


def _dot_nt(a, b):
    return lax.dot_general(a, b, (((1,), (1,)), ((), ())), preferred_element_type=F32)


def _aligned(start, size):
    return pl.ds(pl.multiple_of(start, size), size)


def _kernel(
    ax_h, k_h, v_h, wq_h, wo_h, bx_h, ckv_h, bwq_h, wuk_h, wuv_h, bwo_h,
    out_ref,
    ax_v, bx_v, k_v, v_v, wq_v, wo_v, ckv_v, bwq_v, wuk_v, wuv_v, bwo_v,
    e_v, et_v, l_v, s_v, qa_v, p_v, o_v, ctx_v,
):
    H, W, D = k_v.shape
    M = wo_v.shape[1]
    SK_B, C = ckv_v.shape
    n_cw = LANES * H // CW
    n_kb = SK_B // KB
    scale = float(D) ** -0.5
    window = pl.ds(k_h.shape[2] - W, W)

    copies = [
        (bwq_h, bwq_v),
        (bx_h, bx_v),
        (ax_h, ax_v),
        (wuk_h, wuk_v),
        (ckv_h.at[0], ckv_v),
        (wq_h, wq_v),
        (k_h.at[0, :, window], k_v),
        (wuv_h, wuv_v),
        (v_h.at[0, :, window], v_v),
        (bwo_h, bwo_v),
    ]
    wo_rows = []
    for nh in WO_SPLIT:
        wo_rows.append((sum(n for _, n in wo_rows), nh * D))

    def diag_mask(rows):
        r = lax.broadcasted_iota(jnp.int32, (rows, CW), 0)
        c = lax.broadcasted_iota(jnp.int32, (rows, CW), 1)
        return (r % H) == (c % H)

    def expand(y):
        ys = jnp.concatenate(
            [y[:, j:j + LANES] for j in range(0, y.shape[1], LANES)], axis=0)

        @pl.loop(0, n_cw)
        def _(i):
            l_v[i] = jnp.where(diag_mask(ys.shape[0]), _dot(ys, et_v[i]), 0.0).astype(BF)

    def head_contract(w_v):
        def body(t, acc):
            lhs = l_v[t % n_cw, _aligned(t // n_cw * H, H), :]
            return acc + _dot(lhs, w_v[_aligned(t * CW, CW), :])

        return lax.fori_loop(0, w_v.shape[0] // CW, body, jnp.zeros((H, D), F32))

    def run(sems, wo_sems):
        (bwq_c, bx_c, ax_c, wuk_c, ckv_c, wq_c, k_c, wuv_c, v_c, bwo_c) = dmas = [
            pltpu.make_async_copy(src, dst, sems.at[i])
            for i, (src, dst) in enumerate(copies)
        ]
        wo_dmas = [
            pltpu.make_async_copy(
                wo_h.at[pl.ds(r0, n)], wo_v.at[pl.ds(r0, n)], wo_sems.at[i])
            for i, (r0, n) in enumerate(wo_rows)
        ]
        for dma in dmas:
            dma.start()

        @pl.loop(0, n_cw)
        def _(i):
            r = lax.broadcasted_iota(jnp.int32, (CW, LANES), 0) + i * CW
            c = lax.broadcasted_iota(jnp.int32, (CW, LANES), 1)
            e_v[i] = jnp.where(lax.div(r, H) == c, 1.0, 0.0).astype(BF)
            r = lax.broadcasted_iota(jnp.int32, (LANES, CW), 1) + i * CW
            c = lax.broadcasted_iota(jnp.int32, (LANES, CW), 0)
            et_v[i] = jnp.where(lax.div(r, H) == c, 1.0, 0.0).astype(BF)

        for dma in wo_dmas:
            dma.start()

        bwq_c.wait()
        bx_c.wait()
        expand(jnp.broadcast_to(bx_v[0].astype(F32), (H, M)).astype(BF))
        qb = head_contract(bwq_v).astype(BF)

        ax_c.wait()
        wuk_c.wait()

        @pl.loop(0, wuk_v.shape[0] // CW)
        def _(t):
            r = _dot_nt(qb, wuk_v[_aligned(t * CW, CW), :])
            l_v[t % n_cw, _aligned(t // n_cw * H, H), :] = (
                jnp.where(diag_mask(H), r, 0.0).astype(BF))

        qs = lax.fori_loop(
            0, n_cw, lambda i, acc: acc + _dot(l_v[i], e_v[i]),
            jnp.zeros((l_v.shape[1], LANES), F32)).astype(BF)
        q_abs = jnp.concatenate([qs[j:j + H] for j in range(0, qs.shape[0], H)], axis=1)

        ckv_c.wait()

        def scores_b(i, m):
            s = _dot_nt(q_abs, ckv_v[_aligned(i * KB, KB), :]) * scale
            s_v[i] = s
            for j in range(0, KB, LANES):
                m = jnp.maximum(m, s[:, j:j + LANES])
            return m

        m = lax.fori_loop(0, n_kb, scores_b, jnp.full((H, LANES), -jnp.inf, F32))
        m = jnp.max(m, axis=1, keepdims=True)

        def pv_b(i, carry):
            denom, acc = carry
            p = jnp.exp(s_v[i] - m)
            for j in range(0, KB, LANES):
                denom = denom + p[:, j:j + LANES]
            return denom, acc + _dot(p.astype(BF), ckv_v[_aligned(i * KB, KB), :])

        denom, acc = lax.fori_loop(
            0, n_kb, pv_b, (jnp.zeros((H, LANES), F32), jnp.zeros((H, C), F32)))
        expand((acc / jnp.sum(denom, axis=1, keepdims=True)).astype(BF))

        wq_c.wait()
        xa = jnp.broadcast_to(ax_v[0].astype(F32), (8, M)).astype(BF)

        @pl.loop(0, H // 4)
        def _(i):
            q = _dot(xa, wq_v[:, _aligned(i * 4 * D, 4 * D)])
            for j in range(4):
                qa_v[i * 4 + j] = q[:, j * D:(j + 1) * D]

        k_c.wait()

        @pl.loop(0, H, unroll=2)
        def _(h):
            s = _dot_nt(qa_v[h].astype(BF), k_v[h]) * scale
            p = jnp.exp(s - jnp.max(s, axis=1, keepdims=True))
            p_v[h] = p / jnp.sum(p, axis=1, keepdims=True)

        wuv_c.wait()
        ctx_v[...] = head_contract(wuv_v)

        v_c.wait()

        @pl.loop(0, H, unroll=2)
        def _(h):
            o_v[:, _aligned(h * D, D)] = _dot(p_v[h].astype(BF), v_v[h])

        bwo_c.wait()

        def out_b(g, acc):
            rows = ctx_v[_aligned(g * 8, 8), :]
            lhs = jnp.concatenate(
                [jnp.broadcast_to(rows[j:j + 1], (8, D)) for j in range(8)], axis=1)
            return acc + _dot(lhs.astype(BF), bwo_v[_aligned(g * 8 * D, 8 * D), :])

        ob = lax.fori_loop(0, H // 8, out_b, jnp.zeros((8, M), F32))
        out_ref[0, :, M:] = ob[0:1].astype(out_ref.dtype)

        def out_a(rows, acc):
            return acc + _dot(o_v[:, rows].astype(BF), wo_v[rows, :])

        oa = jnp.zeros((8, M), F32)
        step = 4 * D
        for dma, (r0, n) in zip(wo_dmas, wo_rows):
            dma.wait()
            if n > step:
                oa = lax.fori_loop(
                    r0 // step, (r0 + n) // step,
                    lambda t, acc: out_a(_aligned(t * step, step), acc), oa)
            else:
                oa = out_a(pl.ds(r0, n), oa)
        out_ref[0, :, :M] = oa[0:1].astype(out_ref.dtype)

    pl.run_scoped(
        run,
        pltpu.SemaphoreType.DMA((len(copies),)),
        pltpu.SemaphoreType.DMA((len(wo_rows),)),
    )


@jax.jit
def pallas_concat_heads__sliding_block_cached__compressed_kv_cla__decode_kernel(
    A_x: jax.Array,
    A_k_cache: jax.Array,
    A_v_cache: jax.Array,
    A_wq: jax.Array,
    A_wo: jax.Array,
    B_x: jax.Array,
    B_c_kv: jax.Array,
    B_w_q: jax.Array,
    B_w_uk: jax.Array,
    B_w_uv: jax.Array,
    B_w_o: jax.Array,
):
    M = A_x.shape[-1]
    _, H, SK_A, D = A_k_cache.shape
    W = min(4096, max(256, SK_A // 4))
    _, SK_B, C = B_c_kv.shape
    assert A_x.shape == B_x.shape == (1, 1, M) and M == C == 4 * LANES
    assert B_w_q.shape == (M, H, D) and B_w_uk.shape == B_w_uv.shape == (C, H, D)
    assert D == LANES and sum(WO_SPLIT) == H
    n_cw = LANES * H // CW

    return pl.pallas_call(
        _kernel,
        out_shape=jax.ShapeDtypeStruct((1, 1, 2 * M), A_x.dtype),
        in_specs=[pl.BlockSpec(memory_space=pltpu.HBM)] * 11,
        out_specs=pl.BlockSpec(memory_space=pltpu.VMEM),
        scratch_shapes=[
            pltpu.VMEM((1, 1, M), BF),
            pltpu.VMEM((1, 1, M), BF),
            pltpu.VMEM((H, W, D), BF),
            pltpu.VMEM((H, W, D), BF),
            pltpu.VMEM((M, H * D), BF),
            pltpu.VMEM((H * D, M), BF),
            pltpu.VMEM((SK_B, C), BF),
            pltpu.VMEM((M * H, D), BF),
            pltpu.VMEM((C * H, D), BF),
            pltpu.VMEM((C * H, D), BF),
            pltpu.VMEM((H * D, M), BF),
            pltpu.VMEM((n_cw, CW, LANES), BF),
            pltpu.VMEM((n_cw, LANES, CW), BF),
            pltpu.VMEM((n_cw, C // LANES * H, CW), BF),
            pltpu.VMEM((SK_B // KB, H, KB), F32),
            pltpu.VMEM((H, 8, D), F32),
            pltpu.VMEM((H, 8, W), F32),
            pltpu.VMEM((8, H * D), F32),
            pltpu.VMEM((H, D), F32),
        ],
        compiler_params=pltpu.CompilerParams(vmem_limit_bytes=64 * 1024 * 1024),
    )(
        A_x, A_k_cache, A_v_cache, A_wq, A_wo, B_x, B_c_kv,
        B_w_q.reshape(M * H, D),
        B_w_uk.reshape(C * H, D),
        B_w_uv.reshape(C * H, D),
        B_w_o.reshape(H * D, M),
    )
```

```python
import jax
import jax.numpy as jnp
from jax import lax
import jax.experimental.pallas as pl
import jax.experimental.pallas.tpu as pltpu

BF = jnp.bfloat16
F32 = jnp.float32
LANES = 128
CW = 1024
KB = 512
WO_MXU_ROWS = (2048, 1024, 512, 256)
WO_VPU_ROWS = (128, 96, 32)


def _dot(a, b):
    return jnp.dot(a, b, preferred_element_type=F32)


def _dot_nt(a, b):
    return lax.dot_general(a, b, (((1,), (1,)), ((), ())), preferred_element_type=F32)


def _aligned(start, size):
    return pl.ds(pl.multiple_of(start, size), size)


def _kernel(
    ax_h, k_h, v_h, wq_h, wo_h, bx_h, ckv_h, bwq_h, wuk_h, wuv_h, bwo_h,
    out_ref,
    ax_v, bx_v, k_v, v_v, wq_v, wo_v, ckv_v, bwq_v, wuk_v, wuv_v, bwo_v,
    e_v, et_v, l_v, s_v, qa_v, p_v, o_v, ctx_v, ot_v,
):
    H, W, D = k_v.shape
    M = wo_v.shape[1]
    SK_B, C = ckv_v.shape
    n_cw = LANES * H // CW
    n_kb = SK_B // KB
    scale = float(D) ** -0.5
    window = pl.ds(k_h.shape[2] - W, W)

    copies = [
        (bwq_h, bwq_v),
        (bx_h, bx_v),
        (ax_h, ax_v),
        (wuk_h, wuk_v),
        (ckv_h.at[0], ckv_v),
        (wq_h, wq_v),
        (k_h.at[0, :, window], k_v),
        (wuv_h, wuv_v),
        (v_h.at[0, :, window], v_v),
        (bwo_h, bwo_v),
    ]
    wo_rows = []
    for n in WO_MXU_ROWS + WO_VPU_ROWS:
        r0 = sum(size for _, size in wo_rows)
        wo_rows.append((r0, n))
        copies.append((wo_h.at[pl.ds(r0, n)], wo_v.at[pl.ds(r0, n)]))

    def diag_mask(rows):
        r = lax.broadcasted_iota(jnp.int32, (rows, CW), 0)
        c = lax.broadcasted_iota(jnp.int32, (rows, CW), 1)
        return (r % H) == (c % H)

    def expand(y):
        ys = jnp.concatenate(
            [y[:, j:j + LANES] for j in range(0, y.shape[1], LANES)], axis=0)

        @pl.loop(0, n_cw)
        def _(i):
            l_v[i] = jnp.where(diag_mask(ys.shape[0]), _dot(ys, et_v[i]), 0.0).astype(BF)

    def head_contract(w_v):
        def body(t, acc):
            lhs = l_v[t % n_cw, _aligned(t // n_cw * H, H), :]
            return acc + _dot(lhs, w_v[_aligned(t * CW, CW), :])

        return lax.fori_loop(0, w_v.shape[0] // CW, body, jnp.zeros((H, D), F32))

    def run(sems):
        dmas = [
            pltpu.make_async_copy(src, dst, sems.at[i])
            for i, (src, dst) in enumerate(copies)
        ]
        for dma in dmas:
            dma.start()
        bwq_c, bx_c, ax_c, wuk_c, ckv_c, wq_c, k_c, wuv_c, v_c, bwo_c, *wo_c = dmas

        @pl.loop(0, n_cw)
        def _(i):
            r = lax.broadcasted_iota(jnp.int32, (CW, LANES), 0) + i * CW
            c = lax.broadcasted_iota(jnp.int32, (CW, LANES), 1)
            e_v[i] = jnp.where(r // H == c, 1.0, 0.0).astype(BF)
            r = lax.broadcasted_iota(jnp.int32, (LANES, CW), 1) + i * CW
            c = lax.broadcasted_iota(jnp.int32, (LANES, CW), 0)
            et_v[i] = jnp.where(r // H == c, 1.0, 0.0).astype(BF)

        bwq_c.wait()
        bx_c.wait()
        expand(jnp.broadcast_to(bx_v[0].astype(F32), (H, M)).astype(BF))
        qb = head_contract(bwq_v).astype(BF)

        ax_c.wait()
        wuk_c.wait()

        @pl.loop(0, wuk_v.shape[0] // CW)
        def _(t):
            r = _dot_nt(qb, wuk_v[_aligned(t * CW, CW), :])
            l_v[t % n_cw, _aligned(t // n_cw * H, H), :] = (
                jnp.where(diag_mask(H), r, 0.0).astype(BF))

        qs = lax.fori_loop(
            0, n_cw, lambda i, acc: acc + _dot(l_v[i], e_v[i]),
            jnp.zeros((l_v.shape[1], LANES), F32)).astype(BF)
        q_abs = jnp.concatenate([qs[j:j + H] for j in range(0, qs.shape[0], H)], axis=1)

        ckv_c.wait()

        def scores_b(i, m):
            s = _dot_nt(q_abs, ckv_v[_aligned(i * KB, KB), :]) * scale
            s_v[i] = s
            for j in range(0, KB, LANES):
                m = jnp.maximum(m, s[:, j:j + LANES])
            return m

        m = lax.fori_loop(0, n_kb, scores_b, jnp.full((H, LANES), -jnp.inf, F32))
        m = jnp.max(m, axis=1, keepdims=True)

        def pv_b(i, carry):
            denom, acc = carry
            p = jnp.exp(s_v[i] - m)
            for j in range(0, KB, LANES):
                denom = denom + p[:, j:j + LANES]
            return denom, acc + _dot(p.astype(BF), ckv_v[_aligned(i * KB, KB), :])

        denom, acc = lax.fori_loop(
            0, n_kb, pv_b, (jnp.zeros((H, LANES), F32), jnp.zeros((H, C), F32)))
        expand((acc / jnp.sum(denom, axis=1, keepdims=True)).astype(BF))

        wq_c.wait()
        xa = jnp.broadcast_to(ax_v[0].astype(F32), (8, M)).astype(BF)

        @pl.loop(0, H // 4)
        def _(i):
            q = _dot(xa, wq_v[:, _aligned(i * 4 * D, 4 * D)])
            for j in range(4):
                qa_v[i * 4 + j] = q[:, j * D:(j + 1) * D]

        k_c.wait()

        @pl.loop(0, H, unroll=2)
        def _(h):
            s = _dot_nt(qa_v[h].astype(BF), k_v[h]) * scale
            p = jnp.exp(s - jnp.max(s, axis=1, keepdims=True))
            p_v[h] = p / jnp.sum(p, axis=1, keepdims=True)

        wuv_c.wait()
        ctx_v[...] = head_contract(wuv_v)

        v_c.wait()

        @pl.loop(0, H, unroll=2)
        def _(h):
            o_v[:, _aligned(h * D, D)] = _dot(p_v[h].astype(BF), v_v[h])

        bwo_c.wait()

        def out_b(g, acc):
            rows = ctx_v[_aligned(g * 8, 8), :]
            lhs = jnp.concatenate(
                [jnp.broadcast_to(rows[j:j + 1], (8, D)) for j in range(8)], axis=1)
            return acc + _dot(lhs.astype(BF), bwo_v[_aligned(g * 8 * D, 8 * D), :])

        ob = lax.fori_loop(0, H // 8, out_b, jnp.zeros((8, M), F32))
        out_ref[0, :, M:] = ob[0:1].astype(out_ref.dtype)

        last = sum(WO_MXU_ROWS)
        for r in range(last, H * D, LANES):
            o = o_v[0:1, r:r + LANES].astype(BF).astype(F32)
            ot_v[r - last:r - last + LANES, :] = jnp.broadcast_to(o, (LANES, LANES)).T

        def out_a(rows, acc):
            return acc + _dot(o_v[:, rows].astype(BF), wo_v[rows, :])

        pieces = list(zip(wo_c, wo_rows))
        oa = jnp.zeros((8, M), F32)
        step = 4 * D
        for dma, (r0, n) in pieces[:len(WO_MXU_ROWS)]:
            dma.wait()
            if n > step:
                oa = lax.fori_loop(
                    r0 // step, (r0 + n) // step,
                    lambda t, acc: out_a(_aligned(t * step, step), acc), oa)
            else:
                oa = out_a(pl.ds(r0, n), oa)

        oa = jnp.where(lax.broadcasted_iota(jnp.int32, oa.shape, 0) == 0, oa, 0.0)
        for dma, (r0, n) in pieces[len(WO_MXU_ROWS):]:
            dma.wait()
            for r1 in range(r0, r0 + n, 32):
                t = [
                    wo_v[r:r + 8, :].astype(F32)
                    * jnp.concatenate([ot_v[r - last:r - last + 8, :]] * (M // LANES), axis=1)
                    for r in range(r1, r1 + 32, 8)
                ]
                oa = oa + ((t[0] + t[1]) + (t[2] + t[3]))
        out_ref[0, :, :M] = jnp.sum(oa, axis=0, keepdims=True).astype(out_ref.dtype)

    pl.run_scoped(run, pltpu.SemaphoreType.DMA((len(copies),)))


@jax.jit
def pallas_concat_heads__sliding_block_cached__compressed_kv_cla__decode_kernel(
    A_x: jax.Array,
    A_k_cache: jax.Array,
    A_v_cache: jax.Array,
    A_wq: jax.Array,
    A_wo: jax.Array,
    B_x: jax.Array,
    B_c_kv: jax.Array,
    B_w_q: jax.Array,
    B_w_uk: jax.Array,
    B_w_uv: jax.Array,
    B_w_o: jax.Array,
):
    M = A_x.shape[-1]
    _, H, SK_A, D = A_k_cache.shape
    W = min(4096, max(256, SK_A // 4))
    _, SK_B, C = B_c_kv.shape
    assert A_x.shape == B_x.shape == (1, 1, M) and M == C == 4 * LANES
    assert B_w_q.shape == (M, H, D) and B_w_uk.shape == B_w_uv.shape == (C, H, D)
    assert D == LANES and sum(WO_MXU_ROWS + WO_VPU_ROWS) == H * D
    n_cw = LANES * H // CW

    return pl.pallas_call(
        _kernel,
        out_shape=jax.ShapeDtypeStruct((1, 1, 2 * M), A_x.dtype),
        in_specs=[pl.BlockSpec(memory_space=pltpu.HBM)] * 11,
        out_specs=pl.BlockSpec(memory_space=pltpu.VMEM),
        scratch_shapes=[
            pltpu.VMEM((1, 1, M), BF),
            pltpu.VMEM((1, 1, M), BF),
            pltpu.VMEM((H, W, D), BF),
            pltpu.VMEM((H, W, D), BF),
            pltpu.VMEM((M, H * D), BF),
            pltpu.VMEM((H * D, M), BF),
            pltpu.VMEM((SK_B, C), BF),
            pltpu.VMEM((M * H, D), BF),
            pltpu.VMEM((C * H, D), BF),
            pltpu.VMEM((C * H, D), BF),
            pltpu.VMEM((H * D, M), BF),
            pltpu.VMEM((n_cw, CW, LANES), BF),
            pltpu.VMEM((n_cw, LANES, CW), BF),
            pltpu.VMEM((n_cw, C // LANES * H, CW), BF),
            pltpu.VMEM((SK_B // KB, H, KB), F32),
            pltpu.VMEM((H, 8, D), F32),
            pltpu.VMEM((H, 8, W), F32),
            pltpu.VMEM((8, H * D), F32),
            pltpu.VMEM((H, D), F32),
            pltpu.VMEM((sum(WO_VPU_ROWS), LANES), F32),
        ],
        compiler_params=pltpu.CompilerParams(vmem_limit_bytes=64 * 1024 * 1024),
    )(
        A_x, A_k_cache, A_v_cache, A_wq, A_wo, B_x, B_c_kv,
        B_w_q.reshape(M * H, D),
        B_w_uk.reshape(C * H, D),
        B_w_uv.reshape(C * H, D),
        B_w_o.reshape(H * D, M),
    )
```

```python
import jax
import jax.numpy as jnp
from jax import lax
import jax.experimental.pallas as pl
import jax.experimental.pallas.tpu as pltpu

BF = jnp.bfloat16
F32 = jnp.float32
LANES = 128
CW = 1024
KB = 512
WO_MXU_ROWS = (2048, 1024, 512, 256)
WO_VPU_ROWS = (128, 96, 32)
RELAY_BLOCKS = 9
RELAY_ROWS = 128


def _dot(a, b):
    return jnp.dot(a, b, preferred_element_type=F32)


def _dot_nt(a, b):
    return lax.dot_general(a, b, (((1,), (1,)), ((), ())), preferred_element_type=F32)


def _aligned(start, size):
    return pl.ds(pl.multiple_of(start, size), size)


def _kernel(
    ax_h, k_h, v_h, wq_h, wo_h, bx_h, ckv_h, bwq_h, wuk_h, wuv_h, bwo_h,
    out_ref,
    ax_v, bx_v, k_v, v_v, wq_v, wo_v, ckv_v, bwq_v, wuk_v, wuv_v, bwo_v,
    e_v, et_v, l_v, s_v, qa_v, p_v, o_v, ctx_v, ot_v, *relay_s,
):
    H, W, D = k_v.shape
    M = wo_v.shape[1]
    SK_B, C = ckv_v.shape
    n_cw = LANES * H // CW
    n_kb = SK_B // KB
    scale = float(D) ** -0.5
    window = pl.ds(k_h.shape[2] - W, W)
    lo, hi = pl.ds(0, H // 2), pl.ds(H // 2, H // 2)

    copies = [
        (bwq_h, bwq_v),
        (bx_h, bx_v),
        (ax_h, ax_v),
        (wuk_h, wuk_v),
        (ckv_h.at[0], ckv_v),
        (wq_h, wq_v),
        (k_h.at[0, lo, window], k_v.at[lo]),
        (k_h.at[0, hi, window], k_v.at[hi]),
        (wuv_h, wuv_v),
        (v_h.at[0, lo, window], v_v.at[lo]),
        (v_h.at[0, hi, window], v_v.at[hi]),
        (bwo_h, bwo_v),
    ]
    wo_rows = []
    for n in WO_MXU_ROWS + WO_VPU_ROWS:
        r0 = sum(size for _, size in wo_rows)
        wo_rows.append((r0, n))
        start = max(r0, RELAY_BLOCKS * RELAY_ROWS)
        rows = pl.ds(start, r0 + n - start)
        copies.append((wo_h.at[rows], wo_v.at[rows]))

    def diag_mask(rows):
        r = lax.broadcasted_iota(jnp.int32, (rows, CW), 0)
        c = lax.broadcasted_iota(jnp.int32, (rows, CW), 1)
        return (r % H) == (c % H)

    def expand(y):
        ys = jnp.concatenate(
            [y[:, j:j + LANES] for j in range(0, y.shape[1], LANES)], axis=0)

        @pl.loop(0, n_cw)
        def _(i):
            l_v[i] = jnp.where(diag_mask(ys.shape[0]), _dot(ys, et_v[i]), 0.0).astype(BF)

    def head_contract(w_v):
        def body(t, acc):
            lhs = l_v[t % n_cw, _aligned(t // n_cw * H, H), :]
            return acc + _dot(lhs, w_v[_aligned(t * CW, CW), :])

        return lax.fori_loop(0, w_v.shape[0] // CW, body, jnp.zeros((H, D), F32))

    def run(sems, relay_sems):
        dmas = [
            pltpu.make_async_copy(src, dst, sems.at[i])
            for i, (src, dst) in enumerate(copies)
        ]
        for dma in dmas:
            dma.start()
        (bwq_c, bx_c, ax_c, wuk_c, ckv_c, wq_c, k_lo_c, k_hi_c, wuv_c, v_lo_c, v_hi_c,
         bwo_c, *wo_c) = dmas

        def hops(i):
            rows = pl.ds(i * RELAY_ROWS, RELAY_ROWS)
            buf, sem = relay_s[i % 2], relay_sems.at[i % 2]
            return (pltpu.make_async_copy(wo_h.at[rows], buf, sem),
                    pltpu.make_async_copy(buf, wo_v.at[rows], sem))

        def relay(i):
            if 0 <= i - 1 < RELAY_BLOCKS:
                hops(i - 1)[0].wait()
                hops(i - 1)[1].start()
            if 0 <= i - 2 < RELAY_BLOCKS:
                hops(i - 2)[1].wait()
            if i < RELAY_BLOCKS:
                hops(i)[0].start()

        relay(0)

        @pl.loop(0, n_cw)
        def _(i):
            r = lax.broadcasted_iota(jnp.int32, (CW, LANES), 0) + i * CW
            c = lax.broadcasted_iota(jnp.int32, (CW, LANES), 1)
            e_v[i] = jnp.where(r // H == c, 1.0, 0.0).astype(BF)
            r = lax.broadcasted_iota(jnp.int32, (LANES, CW), 1) + i * CW
            c = lax.broadcasted_iota(jnp.int32, (LANES, CW), 0)
            et_v[i] = jnp.where(r // H == c, 1.0, 0.0).astype(BF)

        bwq_c.wait()
        bx_c.wait()
        relay(1)
        expand(jnp.broadcast_to(bx_v[0].astype(F32), (H, M)).astype(BF))
        qb = head_contract(bwq_v).astype(BF)

        ax_c.wait()
        wuk_c.wait()
        relay(2)

        @pl.loop(0, wuk_v.shape[0] // CW)
        def _(t):
            r = _dot_nt(qb, wuk_v[_aligned(t * CW, CW), :])
            l_v[t % n_cw, _aligned(t // n_cw * H, H), :] = (
                jnp.where(diag_mask(H), r, 0.0).astype(BF))

        qs = lax.fori_loop(
            0, n_cw, lambda i, acc: acc + _dot(l_v[i], e_v[i]),
            jnp.zeros((l_v.shape[1], LANES), F32)).astype(BF)
        q_abs = jnp.concatenate([qs[j:j + H] for j in range(0, qs.shape[0], H)], axis=1)

        ckv_c.wait()
        relay(3)

        def scores_b(i, m):
            s = _dot_nt(q_abs, ckv_v[_aligned(i * KB, KB), :]) * scale
            s_v[i] = s
            for j in range(0, KB, LANES):
                m = jnp.maximum(m, s[:, j:j + LANES])
            return m

        m = lax.fori_loop(0, n_kb, scores_b, jnp.full((H, LANES), -jnp.inf, F32))
        m = jnp.max(m, axis=1, keepdims=True)

        def pv_b(i, carry):
            denom, acc = carry
            p = jnp.exp(s_v[i] - m)
            for j in range(0, KB, LANES):
                denom = denom + p[:, j:j + LANES]
            return denom, acc + _dot(p.astype(BF), ckv_v[_aligned(i * KB, KB), :])

        denom, acc = lax.fori_loop(
            0, n_kb, pv_b, (jnp.zeros((H, LANES), F32), jnp.zeros((H, C), F32)))
        expand((acc / jnp.sum(denom, axis=1, keepdims=True)).astype(BF))

        wq_c.wait()
        relay(4)
        xa = jnp.broadcast_to(ax_v[0].astype(F32), (8, M)).astype(BF)

        @pl.loop(0, H // 4)
        def _(i):
            q = _dot(xa, wq_v[:, _aligned(i * 4 * D, 4 * D)])
            for j in range(4):
                qa_v[i * 4 + j] = q[:, j * D:(j + 1) * D]

        def softmax_a(h):
            s = _dot_nt(qa_v[h].astype(BF), k_v[h]) * scale
            p = jnp.exp(s - jnp.max(s, axis=1, keepdims=True))
            p_v[h] = p / jnp.sum(p, axis=1, keepdims=True)

        k_lo_c.wait()
        relay(5)
        pl.loop(0, H // 2, unroll=2)(softmax_a)
        k_hi_c.wait()
        relay(6)
        pl.loop(H // 2, H, unroll=2)(softmax_a)

        wuv_c.wait()
        relay(7)
        ctx_v[...] = head_contract(wuv_v)

        def pv_a(h):
            o_v[:, _aligned(h * D, D)] = _dot(p_v[h].astype(BF), v_v[h])

        v_lo_c.wait()
        relay(8)
        pl.loop(0, H // 2, unroll=2)(pv_a)
        v_hi_c.wait()
        relay(9)
        pl.loop(H // 2, H, unroll=2)(pv_a)

        bwo_c.wait()

        def out_b(g, acc):
            rows = ctx_v[_aligned(g * 8, 8), :]
            lhs = jnp.concatenate(
                [jnp.broadcast_to(rows[j:j + 1], (8, D)) for j in range(8)], axis=1)
            return acc + _dot(lhs.astype(BF), bwo_v[_aligned(g * 8 * D, 8 * D), :])

        ob = lax.fori_loop(0, H // 8, out_b, jnp.zeros((8, M), F32))
        out_ref[0, :, M:] = ob[0:1].astype(out_ref.dtype)

        last = sum(WO_MXU_ROWS)
        for r in range(last, H * D, LANES):
            o = o_v[0:1, r:r + LANES].astype(BF).astype(F32)
            ot_v[r - last:r - last + LANES, :] = jnp.broadcast_to(o, (LANES, LANES)).T

        def out_a(rows, acc):
            return acc + _dot(o_v[:, rows].astype(BF), wo_v[rows, :])

        relay(10)
        pieces = list(zip(wo_c, wo_rows))
        oa = jnp.zeros((8, M), F32)
        step = 4 * D
        for dma, (r0, n) in pieces[:len(WO_MXU_ROWS)]:
            dma.wait()
            if n > step:
                oa = lax.fori_loop(
                    r0 // step, (r0 + n) // step,
                    lambda t, acc: out_a(_aligned(t * step, step), acc), oa)
            else:
                oa = out_a(pl.ds(r0, n), oa)

        oa = jnp.where(lax.broadcasted_iota(jnp.int32, oa.shape, 0) == 0, oa, 0.0)
        for dma, (r0, n) in pieces[len(WO_MXU_ROWS):]:
            dma.wait()
            for r1 in range(r0, r0 + n, 32):
                t = [
                    wo_v[r:r + 8, :].astype(F32)
                    * jnp.concatenate([ot_v[r - last:r - last + 8, :]] * (M // LANES), axis=1)
                    for r in range(r1, r1 + 32, 8)
                ]
                oa = oa + ((t[0] + t[1]) + (t[2] + t[3]))
        out_ref[0, :, :M] = jnp.sum(oa, axis=0, keepdims=True).astype(out_ref.dtype)

    pl.run_scoped(
        run, pltpu.SemaphoreType.DMA((len(copies),)), pltpu.SemaphoreType.DMA((2,)))


@jax.jit
def pallas_concat_heads__sliding_block_cached__compressed_kv_cla__decode_kernel(
    A_x: jax.Array,
    A_k_cache: jax.Array,
    A_v_cache: jax.Array,
    A_wq: jax.Array,
    A_wo: jax.Array,
    B_x: jax.Array,
    B_c_kv: jax.Array,
    B_w_q: jax.Array,
    B_w_uk: jax.Array,
    B_w_uv: jax.Array,
    B_w_o: jax.Array,
):
    M = A_x.shape[-1]
    _, H, SK_A, D = A_k_cache.shape
    W = min(4096, max(256, SK_A // 4))
    _, SK_B, C = B_c_kv.shape
    assert A_x.shape == B_x.shape == (1, 1, M) and M == C == 4 * LANES
    assert B_w_q.shape == (M, H, D) and B_w_uk.shape == B_w_uv.shape == (C, H, D)
    assert D == LANES and sum(WO_MXU_ROWS + WO_VPU_ROWS) == H * D
    assert RELAY_BLOCKS <= 9 and RELAY_BLOCKS * RELAY_ROWS < WO_MXU_ROWS[0]
    n_cw = LANES * H // CW

    return pl.pallas_call(
        _kernel,
        out_shape=jax.ShapeDtypeStruct((1, 1, 2 * M), A_x.dtype),
        in_specs=[pl.BlockSpec(memory_space=pltpu.HBM)] * 11,
        out_specs=pl.BlockSpec(memory_space=pltpu.VMEM),
        scratch_shapes=[
            pltpu.VMEM((1, 1, M), BF),
            pltpu.VMEM((1, 1, M), BF),
            pltpu.VMEM((H, W, D), BF),
            pltpu.VMEM((H, W, D), BF),
            pltpu.VMEM((M, H * D), BF),
            pltpu.VMEM((H * D, M), BF),
            pltpu.VMEM((SK_B, C), BF),
            pltpu.VMEM((M * H, D), BF),
            pltpu.VMEM((C * H, D), BF),
            pltpu.VMEM((C * H, D), BF),
            pltpu.VMEM((H * D, M), BF),
            pltpu.VMEM((n_cw, CW, LANES), BF),
            pltpu.VMEM((n_cw, LANES, CW), BF),
            pltpu.VMEM((n_cw, C // LANES * H, CW), BF),
            pltpu.VMEM((SK_B // KB, H, KB), F32),
            pltpu.VMEM((H, 8, D), F32),
            pltpu.VMEM((H, 8, W), F32),
            pltpu.VMEM((8, H * D), F32),
            pltpu.VMEM((H, D), F32),
            pltpu.VMEM((sum(WO_VPU_ROWS), LANES), F32),
            pltpu.SMEM((RELAY_ROWS, M), BF),
            pltpu.SMEM((RELAY_ROWS, M), BF),
        ],
        compiler_params=pltpu.CompilerParams(vmem_limit_bytes=64 * 1024 * 1024),
    )(
        A_x, A_k_cache, A_v_cache, A_wq, A_wo, B_x, B_c_kv,
        B_w_q.reshape(M * H, D),
        B_w_uk.reshape(C * H, D),
        B_w_uv.reshape(C * H, D),
        B_w_o.reshape(H * D, M),
    )
```

```python
import jax
import jax.numpy as jnp
from jax import lax
import jax.experimental.pallas as pl
import jax.experimental.pallas.tpu as pltpu

BF = jnp.bfloat16
F32 = jnp.float32
LANES = 128
CW = 1024
KB = 512
WO_MXU_ROWS = (2048, 1024, 512, 256)
WO_VPU_ROWS = (128, 96, 32)
RELAY_BLOCKS = 9
RELAY_ROWS = 128


def _dot(a, b):
    return jnp.dot(a, b, preferred_element_type=F32)


def _dot_nt(a, b):
    return lax.dot_general(a, b, (((1,), (1,)), ((), ())), preferred_element_type=F32)


def _aligned(start, size):
    return pl.ds(pl.multiple_of(start, size), size)


def _kernel(
    ax_h, k_h, v_h, wq_h, wo_h, bx_h, ckv_h, bwq_h, wuk_h, wuv_h, bwo_h,
    out_ref,
    ax_v, bx_v, k_v, v_v, wq_v, wo_v, ckv_v, bwq_v, wuk_v, wuv_v, bwo_v,
    e_v, et_v, l_v, s_v, qa_v, p_v, o_v, ctx_v, ot_v, *relay_s,
):
    H, W, D = k_v.shape
    M = wo_v.shape[1]
    SK_B, C = ckv_v.shape
    n_cw = LANES * H // CW
    n_kb = SK_B // KB
    scale = float(D) ** -0.5
    window = pl.ds(k_h.shape[2] - W, W)
    lo, hi = pl.ds(0, H // 2), pl.ds(H // 2, H // 2)

    copies = [
        (bwq_h, bwq_v),
        (bx_h, bx_v),
        (ax_h, ax_v),
        (wuk_h, wuk_v),
        (ckv_h.at[0], ckv_v),
        (wq_h, wq_v),
        (k_h.at[0, lo, window], k_v.at[lo]),
        (k_h.at[0, hi, window], k_v.at[hi]),
        (wuv_h, wuv_v),
        (v_h.at[0, lo, window], v_v.at[lo]),
        (v_h.at[0, hi, window], v_v.at[hi]),
        (bwo_h, bwo_v),
    ]
    wo_rows = []
    for n in WO_MXU_ROWS + WO_VPU_ROWS:
        r0 = sum(size for _, size in wo_rows)
        wo_rows.append((r0, n))
        start = max(r0, RELAY_BLOCKS * RELAY_ROWS)
        rows = pl.ds(start, r0 + n - start)
        copies.append((wo_h.at[rows], wo_v.at[rows]))

    def diag_mask(rows):
        r = lax.broadcasted_iota(jnp.int32, (rows, CW), 0)
        c = lax.broadcasted_iota(jnp.int32, (rows, CW), 1)
        return (r % H) == (c % H)

    def expand(y):
        ys = jnp.concatenate(
            [y[:, j:j + LANES] for j in range(0, y.shape[1], LANES)], axis=0)

        @pl.loop(0, n_cw)
        def _(i):
            l_v[i] = jnp.where(diag_mask(ys.shape[0]), _dot(ys, et_v[i]), 0.0).astype(BF)

    def head_contract(w_v):
        def body(t, acc):
            lhs = l_v[t % n_cw, _aligned(t // n_cw * H, H), :]
            return acc + _dot(lhs, w_v[_aligned(t * CW, CW), :])

        return lax.fori_loop(0, w_v.shape[0] // CW, body, jnp.zeros((H, D), F32))

    def run(sems, relay_sems):
        dmas = [
            pltpu.make_async_copy(src, dst, sems.at[i])
            for i, (src, dst) in enumerate(copies)
        ]
        for dma in dmas:
            dma.start()
        (bwq_c, bx_c, ax_c, wuk_c, ckv_c, wq_c, k_lo_c, k_hi_c, wuv_c, v_lo_c, v_hi_c,
         bwo_c, *wo_c) = dmas

        relay_in, relay_out = [], []
        for i in range(RELAY_BLOCKS):
            rows = pl.ds(i * RELAY_ROWS, RELAY_ROWS)
            buf, sem = relay_s[i % 2], relay_sems.at[i % 2]
            relay_in.append(pltpu.make_async_copy(wo_h.at[rows], buf, sem))
            relay_out.append(pltpu.make_async_copy(buf, wo_v.at[rows], sem))

        def relay(i):
            if 0 <= i - 1 < RELAY_BLOCKS:
                relay_in[i - 1].wait()
                relay_out[i - 1].start()
            if 0 <= i - 2 < RELAY_BLOCKS:
                relay_out[i - 2].wait()
            if i < RELAY_BLOCKS:
                relay_in[i].start()

        relay(0)

        @pl.loop(0, n_cw)
        def _(i):
            r = lax.broadcasted_iota(jnp.int32, (CW, LANES), 0) + i * CW
            c = lax.broadcasted_iota(jnp.int32, (CW, LANES), 1)
            e_v[i] = jnp.where(r // H == c, 1.0, 0.0).astype(BF)
            r = lax.broadcasted_iota(jnp.int32, (LANES, CW), 1) + i * CW
            c = lax.broadcasted_iota(jnp.int32, (LANES, CW), 0)
            et_v[i] = jnp.where(r // H == c, 1.0, 0.0).astype(BF)

        bwq_c.wait()
        bx_c.wait()
        relay(1)
        expand(jnp.broadcast_to(bx_v[0].astype(F32), (H, M)).astype(BF))
        qb = head_contract(bwq_v).astype(BF)

        ax_c.wait()
        wuk_c.wait()
        relay(2)

        @pl.loop(0, wuk_v.shape[0] // CW)
        def _(t):
            r = _dot_nt(qb, wuk_v[_aligned(t * CW, CW), :])
            l_v[t % n_cw, _aligned(t // n_cw * H, H), :] = (
                jnp.where(diag_mask(H), r, 0.0).astype(BF))

        qs = lax.fori_loop(
            0, n_cw, lambda i, acc: acc + _dot(l_v[i], e_v[i]),
            jnp.zeros((l_v.shape[1], LANES), F32)).astype(BF)
        q_abs = jnp.concatenate([qs[j:j + H] for j in range(0, qs.shape[0], H)], axis=1)

        ckv_c.wait()
        relay(3)

        def scores_b(i, m):
            s = _dot_nt(q_abs, ckv_v[_aligned(i * KB, KB), :]) * scale
            s_v[i] = s
            for j in range(0, KB, LANES):
                m = jnp.maximum(m, s[:, j:j + LANES])
            return m

        m = lax.fori_loop(0, n_kb, scores_b, jnp.full((H, LANES), -jnp.inf, F32))
        m = jnp.max(m, axis=1, keepdims=True)

        def pv_b(i, carry):
            denom, acc = carry
            p = jnp.exp(s_v[i] - m)
            for j in range(0, KB, LANES):
                denom = denom + p[:, j:j + LANES]
            return denom, acc + _dot(p.astype(BF), ckv_v[_aligned(i * KB, KB), :])

        denom, acc = lax.fori_loop(
            0, n_kb, pv_b, (jnp.zeros((H, LANES), F32), jnp.zeros((H, C), F32)))
        expand((acc / jnp.sum(denom, axis=1, keepdims=True)).astype(BF))

        wq_c.wait()
        relay(4)
        xa = jnp.broadcast_to(ax_v[0].astype(F32), (8, M)).astype(BF)

        @pl.loop(0, H // 4)
        def _(i):
            q = _dot(xa, wq_v[:, _aligned(i * 4 * D, 4 * D)])
            for j in range(4):
                qa_v[i * 4 + j] = q[:, j * D:(j + 1) * D]

        def softmax_a(h):
            s = _dot_nt(qa_v[h].astype(BF), k_v[h]) * scale
            p = jnp.exp(s - jnp.max(s, axis=1, keepdims=True))
            p_v[h] = p / jnp.sum(p, axis=1, keepdims=True)

        k_lo_c.wait()
        relay(5)
        pl.loop(0, H // 2, unroll=2)(softmax_a)
        k_hi_c.wait()
        relay(6)
        pl.loop(H // 2, H, unroll=2)(softmax_a)

        wuv_c.wait()
        relay(7)
        ctx_v[...] = head_contract(wuv_v)

        def pv_a(h):
            o_v[:, _aligned(h * D, D)] = _dot(p_v[h].astype(BF), v_v[h])

        v_lo_c.wait()
        relay(8)
        pl.loop(0, H // 2, unroll=2)(pv_a)
        v_hi_c.wait()
        relay(9)
        pl.loop(H // 2, H, unroll=2)(pv_a)

        bwo_c.wait()

        def out_b(g, acc):
            rows = ctx_v[_aligned(g * 8, 8), :]
            lhs = jnp.concatenate(
                [jnp.broadcast_to(rows[j:j + 1], (8, D)) for j in range(8)], axis=1)
            return acc + _dot(lhs.astype(BF), bwo_v[_aligned(g * 8 * D, 8 * D), :])

        ob = lax.fori_loop(0, H // 8, out_b, jnp.zeros((8, M), F32))
        out_ref[0, :, M:] = ob[0:1].astype(out_ref.dtype)

        last = sum(WO_MXU_ROWS)
        for r in range(last, H * D, LANES):
            o = o_v[0:1, r:r + LANES].astype(BF).astype(F32)
            ot_v[r - last:r - last + LANES, :] = jnp.broadcast_to(o, (LANES, LANES)).T

        def out_a(rows, acc):
            return acc + _dot(o_v[:, rows].astype(BF), wo_v[rows, :])

        relay(10)
        pieces = list(zip(wo_c, wo_rows))
        oa = jnp.zeros((8, M), F32)
        step = 4 * D
        for dma, (r0, n) in pieces[:len(WO_MXU_ROWS)]:
            dma.wait()
            if n > step:
                oa = lax.fori_loop(
                    r0 // step, (r0 + n) // step,
                    lambda t, acc: out_a(_aligned(t * step, step), acc), oa)
            else:
                oa = out_a(pl.ds(r0, n), oa)

        oa = jnp.where(lax.broadcasted_iota(jnp.int32, oa.shape, 0) == 0, oa, 0.0)
        for dma, (r0, n) in pieces[len(WO_MXU_ROWS):]:
            dma.wait()
            for r1 in range(r0, r0 + n, 32):
                t = [
                    wo_v[r:r + 8, :].astype(F32)
                    * jnp.concatenate([ot_v[r - last:r - last + 8, :]] * (M // LANES), axis=1)
                    for r in range(r1, r1 + 32, 8)
                ]
                oa = oa + ((t[0] + t[1]) + (t[2] + t[3]))
        out_ref[0, :, :M] = jnp.sum(oa, axis=0, keepdims=True).astype(out_ref.dtype)

    pl.run_scoped(
        run, pltpu.SemaphoreType.DMA((len(copies),)), pltpu.SemaphoreType.DMA((2,)))


@jax.jit
def pallas_concat_heads__sliding_block_cached__compressed_kv_cla__decode_kernel(
    A_x: jax.Array,
    A_k_cache: jax.Array,
    A_v_cache: jax.Array,
    A_wq: jax.Array,
    A_wo: jax.Array,
    B_x: jax.Array,
    B_c_kv: jax.Array,
    B_w_q: jax.Array,
    B_w_uk: jax.Array,
    B_w_uv: jax.Array,
    B_w_o: jax.Array,
):
    M = A_x.shape[-1]
    _, H, SK_A, D = A_k_cache.shape
    W = min(4096, max(256, SK_A // 4))
    _, SK_B, C = B_c_kv.shape
    assert A_x.shape == B_x.shape == (1, 1, M) and M == C == 4 * LANES
    assert B_w_q.shape == (M, H, D) and B_w_uk.shape == B_w_uv.shape == (C, H, D)
    assert D == LANES and sum(WO_MXU_ROWS + WO_VPU_ROWS) == H * D
    assert RELAY_BLOCKS <= 9 and RELAY_BLOCKS * RELAY_ROWS < WO_MXU_ROWS[0]
    n_cw = LANES * H // CW

    return pl.pallas_call(
        _kernel,
        out_shape=jax.ShapeDtypeStruct((1, 1, 2 * M), A_x.dtype),
        in_specs=[pl.BlockSpec(memory_space=pltpu.HBM)] * 11,
        out_specs=pl.BlockSpec(memory_space=pltpu.VMEM),
        scratch_shapes=[
            pltpu.VMEM((1, 1, M), BF),
            pltpu.VMEM((1, 1, M), BF),
            pltpu.VMEM((H, W, D), BF),
            pltpu.VMEM((H, W, D), BF),
            pltpu.VMEM((M, H * D), BF),
            pltpu.VMEM((H * D, M), BF),
            pltpu.VMEM((SK_B, C), BF),
            pltpu.VMEM((M * H, D), BF),
            pltpu.VMEM((C * H, D), BF),
            pltpu.VMEM((C * H, D), BF),
            pltpu.VMEM((H * D, M), BF),
            pltpu.VMEM((n_cw, CW, LANES), BF),
            pltpu.VMEM((n_cw, LANES, CW), BF),
            pltpu.VMEM((n_cw, C // LANES * H, CW), BF),
            pltpu.VMEM((SK_B // KB, H, KB), F32),
            pltpu.VMEM((H, 8, D), F32),
            pltpu.VMEM((H, 8, W), F32),
            pltpu.VMEM((8, H * D), F32),
            pltpu.VMEM((H, D), F32),
            pltpu.VMEM((sum(WO_VPU_ROWS), LANES), F32),
            pltpu.SMEM((RELAY_ROWS, M), BF),
            pltpu.SMEM((RELAY_ROWS, M), BF),
        ],
        compiler_params=pltpu.CompilerParams(vmem_limit_bytes=64 * 1024 * 1024),
    )(
        A_x, A_k_cache, A_v_cache, A_wq, A_wo, B_x, B_c_kv,
        B_w_q.reshape(M * H, D),
        B_w_uk.reshape(C * H, D),
        B_w_uv.reshape(C * H, D),
        B_w_o.reshape(H * D, M),
    )
```
